```python
import os as _os
_os.environ.setdefault("JAX_PLATFORMS", "cpu")
import jax
import jax.numpy as jnp

def _softmax(x, axis=-1):
    return jax.nn.softmax(x, axis=axis)
def _gelu(x):
    return jax.nn.gelu(x, approximate=True)
def _silu(x):
    return jax.nn.silu(x)
def _sigmoid(x):
    return jax.nn.sigmoid(x)
def _layernorm(x, axis=-1, eps=1e-5):
    m = jnp.mean(x, axis=axis, keepdims=True)
    v = jnp.var(x, axis=axis, keepdims=True)
    return (x - m) / jnp.sqrt(v + eps)
def _scatter_add(tgt, idx, src, axis=0):
    return tgt.at[idx].add(src)
def _segment_sum(src, seg, n):
    return jax.ops.segment_sum(src, seg, n)
class _Rng:
    def __init__(self, key):
        self._k = key
    def _next(self):
        self._k, sub = jax.random.split(self._k)
        return sub
    def normal(self, shape):
        return jax.random.normal(self._next(), shape, dtype=jnp.bfloat16)
    def randint(self, lo, hi, shape):
        return jax.random.randint(self._next(), shape, lo, hi, dtype=jnp.int32)
    def uniform(self, shape, lo=0.0, hi=1.0):
        return jax.random.uniform(self._next(), shape, jnp.bfloat16, lo, hi)
    def permutation(self, n):
        return jax.random.permutation(self._next(), n)


kernel_name = 'gated_mix__compressed_kv_cla__ssm_conv_h3__prompt'

def setup_inputs():
    _rng = _Rng(jax.random.key(int.from_bytes(__import__("os").urandom(4), "little")))
    _w = (lambda a: (lambda t: t.astype(jnp.bfloat16) if jnp.issubdtype(t.dtype, jnp.floating) else t)(jnp.asarray(a)))
    def _A_setup():
        B, H, Sq, Sk, D, M = 1, 32, 2048, 2048, 128, 1024
        Dc = 4 * D
        return {
            "x": _w((lambda *s: _rng.normal(s) * 0.05)(B, Sq, M)),
            "c_kv": _w((lambda *s: _rng.normal(s) * 0.8)(B, Sk, Dc)),
            "w_q": _w((lambda *s: _rng.normal(s) * 3.2)(M, H, D) * (M ** -0.5)),
            "w_uk": _w((lambda *s: _rng.normal(s) * 3.2)(Dc, H, D) * (Dc ** -0.5)),
            "w_uv": _w((lambda *s: _rng.normal(s) * 0.8)(Dc, H, D) * (Dc ** -0.5)),
            "w_o": _w((lambda *s: _rng.normal(s) * 0.8)(H, D, M) * ((H * D) ** -0.5)),
        }
    _A_in = _A_setup()

    def _B_setup():
        B, S, D = 1, 2048, 1024
        ks = 4
        return {
            "q": _w((lambda *s: _rng.normal(s) * 0.05)(B, S, D)),
            "k": _w((lambda *s: _rng.normal(s) * 0.8)(B, S, D)),
            "v": _w((lambda *s: _rng.normal(s) * 0.8)(B, S, D)),
            "shift_k": _w((lambda *s: _rng.normal(s) * 0.8)(D, ks) * 0.5),
            "ssm_k": _w((lambda *s: _rng.normal(s) * 0.8)(D, S) * (1.0 / S ** 0.5)),
            "ssm_D": _w((lambda *s: _rng.normal(s) * 0.8)(D)),
        }
    _B_in = _B_setup()

    return {
        "A_x": _A_in["x"],
        "A_c_kv": _A_in["c_kv"],
        "A_w_q": _A_in["w_q"],
        "A_w_uk": _A_in["w_uk"],
        "A_w_uv": _A_in["w_uv"],
        "A_w_o": _A_in["w_o"],
        "B_q": _B_in["q"],
        "B_k": _B_in["k"],
        "B_v": _B_in["v"],
        "B_shift_k": _B_in["shift_k"],
        "B_ssm_k": _B_in["ssm_k"],
        "B_ssm_D": _B_in["ssm_D"],
        "gate_w": _w((lambda *s: _rng.normal(s) * 0.05)(1024) * 16.0),
    }

def reference(A_x, A_c_kv, A_w_q, A_w_uk, A_w_uv, A_w_o, B_q, B_k, B_v, B_shift_k, B_ssm_k, B_ssm_D, gate_w):
    def _A_ref(x, c_kv, w_q, w_uk, w_uv, w_o):
        B, Sq, M = x.shape[0], x.shape[1], x.shape[2]
        Sk = c_kv.shape[1]
        H, D = w_q.shape[1], w_q.shape[2]
        q = jnp.einsum("bqm,mhd->bhqd", x, w_q)
        k = jnp.einsum("bkc,chd->bhkd", c_kv, w_uk)
        v = jnp.einsum("bkc,chd->bhkd", c_kv, w_uv)
        scores = jnp.einsum("bhqd,bhkd->bhqk", q, k) * (D ** -0.5)
        off = Sk - Sq
        qi = jnp.arange(Sq)[:, None]
        kj = jnp.arange(Sk)[None, :]
        cmask = kj <= (qi + off)
        scores = jnp.where(cmask[None, None], scores, -1e9)
        p = _softmax(scores, axis=-1)
        ctx = jnp.einsum("bhqk,bhkd->bhqd", p, v)
        return jnp.einsum("bhqd,hdm->bqm", ctx, w_o)

    def _B_ref(q, k, v, shift_k, ssm_k, ssm_D):
        B, S, D = q.shape
        ks = shift_k.shape[-1]
        k_pad = jnp.pad(k, ((0, 0), (ks - 1, 0), (0, 0)))
        k_shift = jnp.zeros_like(k)
        for t in range(ks):
            k_shift = k_shift + k_pad[:, t:t + S, :] * shift_k[:, ks - 1 - t][None, None, :]
        kv = k_shift * v
        L = 2 * S
        kv_pad = jnp.pad(kv, ((0, 0), (0, S), (0, 0)))
        kf_pad = jnp.pad(ssm_k, ((0, 0), (0, S)))
        kv_f = (lambda x, axes=(-2,-1): jnp.fft.rfft2(x.astype(jnp.float32), axes=axes))(kv_pad[:, None, :, :], axes=(1, 2))
        kf_f = (lambda x, axes=(-2,-1): jnp.fft.rfft2(x.astype(jnp.float32), axes=axes))(kf_pad[:, None, :], axes=(1, 2))
        kf_f = (lambda x, *d: x.transpose(*d))(kf_f, 1, 2, 0)
        y_f = kv_f * kf_f[None, :, :, :]
        y = (lambda x, s, axes=(-2,-1): jnp.fft.irfft2(x, s=s, axes=axes).astype(jnp.bfloat16))(y_f, (1, L), axes=(1, 2))[:, 0, :S, :]
        y = y + kv * ssm_D[None, None, :]
        return q * y

    x = A_x
    g = _sigmoid((x * gate_w).sum(-1, keepdims=True))
    a = _A_ref(x, A_c_kv, A_w_q, A_w_uk, A_w_uv, A_w_o)
    b = _B_ref(x, B_k, B_v, B_shift_k, B_ssm_k, B_ssm_D)
    return g * a + (1 - g) * b
```

```python
import numpy as np
import jax
import jax.numpy as jnp
from jax import lax
import jax.experimental.pallas as pl
import jax.experimental.pallas.tpu as pltpu

BF = jnp.bfloat16
F32 = jnp.float32
T = 128
LOG2E = 1.4426950408889634
_NT = (((1,), (1,)), ((), ()))


def _dft_matrices():
    f = np.concatenate([np.arange(0, T, 2), np.arange(1, T, 2)]).astype(np.float64)
    ang = np.pi * (f[:, None] + 0.5) * np.arange(T)[None, :] / T
    fwd = np.concatenate([np.cos(ang), -np.sin(ang)], axis=0)
    inv = fwd.T / T
    return fwd.astype(BF), inv.astype(BF)


def _dot(a, b):
    return jnp.dot(a, b, preferred_element_type=F32)


def _dot_nt(a, b):
    return lax.dot_general(a, b, _NT, preferred_element_type=F32)


def _split_pair(u):
    lo = pltpu.bitcast(u << 16, F32)
    hi = pltpu.bitcast(u & jnp.uint32(0xFFFF0000), F32)
    return lo, hi


def _causal_conv(xs, hs):
    out = []
    for a in range(len(xs)):
        acc = xs[a] * hs[0]
        for m in range(1, a + 1):
            acc = acc + xs[a - m] * hs[m]
        out.append(acc)
    return out


def _kernel(shift_ref, d_ref, gw_ref, fwd_ref, inv_ref,
            x_hbm, c_hbm, wq_hbm, wk_hbm, wv_hbm, wo_hbm, bk_hbm, bv_hbm, h_hbm,
            o_hbm,
            x_v, c_v, wq_u, wk_u, wv_u, wq_b, wkv_b, k_s, v_s, ctx_s,
            wo_v, bk_v, bv_v, h_v, g_s, par_s, kpad, o_v,
            sem_x, sem_c, sem_w, sem_b, sem_o):
    NX, S, _ = x_v.shape
    NC = c_v.shape[0]
    H = ctx_s.shape[0]
    NP = H // 2
    NB = S // T
    KS = shift_ref.shape[0]
    qscale = (T ** -0.5) * LOG2E

    def col_copies(hbm, vmem, sem):
        return [pltpu.make_async_copy(hbm.at[:, pl.ds(j * T, T)], vmem.at[j], sem)
                for j in range(vmem.shape[0])]

    def w_copies(p, slot):
        return [pltpu.make_async_copy(hbm.bitcast(jnp.uint32).at[:, p, :], buf.at[slot],
                                      sem_w.at[slot, n])
                for n, (hbm, buf) in enumerate(((wk_hbm, wk_u), (wv_hbm, wv_u), (wq_hbm, wq_u)))]

    c_cp = col_copies(c_hbm, c_v, sem_c)
    x_cp = col_copies(x_hbm, x_v, sem_x)
    b_cp = (col_copies(wo_hbm, wo_v, sem_b.at[0]) + col_copies(bk_hbm, bk_v, sem_b.at[1])
            + col_copies(bv_hbm, bv_v, sem_b.at[2])
            + [pltpu.make_async_copy(h_hbm, h_v, sem_b.at[3])])
    for cp in w_copies(0, 0) + c_cp + x_cp:
        cp.start()

    shift = shift_ref[...].astype(F32)
    dvec = d_ref[...].astype(F32)
    for j in range(NX):
        par_s[j, 0:KS, :] = shift[:, j * T:(j + 1) * T]
        par_s[j, KS:KS + 1, :] = dvec[j:j + 1, :]
    kpad[0:8, :] = jnp.zeros((8, T), F32)

    for cp in c_cp + x_cp:
        cp.wait()
    for cp in b_cp:
        cp.start()

    gw = gw_ref[...].astype(F32)
    for i in range(NB):
        rows = pl.ds(i * T, T)
        acc = x_v[0, rows, :].astype(F32) * gw[0:1, :]
        for j in range(1, NX):
            acc = acc + x_v[j, rows, :].astype(F32) * gw[j:j + 1, :]
        g_s[rows, :] = jnp.broadcast_to(
            jax.nn.sigmoid(jnp.sum(acc, axis=1, keepdims=True)), (T, T))

    def pair_body(p, carry):
        slot = p % 2
        for cp in w_copies(p, slot):
            cp.wait()

        @pl.when(p + 1 < NP)
        def _():
            for cp in w_copies(p + 1, 1 - slot):
                cp.start()

        for n, buf in enumerate((wk_u, wv_u)):
            for e, w in enumerate(_split_pair(buf[slot])):
                wkv_b[:, pl.ds((2 * n + e) * T, T)] = w.astype(BF)
        for e, w in enumerate(_split_pair(wq_u[slot])):
            wq_b[:, pl.ds(e * T, T)] = w.astype(BF)

        RC = 512
        for r in range(S // RC):
            rows = pl.ds(r * RC, RC)
            c = jnp.concatenate([c_v[j, rows, :] for j in range(NC)], axis=1)
            kv = _dot(c, wkv_b[...]).astype(BF)
            for e in range(2):
                k_s[e, rows, :] = kv[:, e * T:(e + 1) * T]
                v_s[e, rows, :] = kv[:, (2 + e) * T:(3 + e) * T]

        row = lax.broadcasted_iota(jnp.int32, (T, T), 0)
        col = lax.broadcasted_iota(jnp.int32, (T, T), 1)

        def q_proj(i):
            xb = jnp.concatenate([x_v[j, pl.ds(i * T, T), :] for j in range(NX)], axis=1)
            return (_dot(xb, wq_b[...]) * qscale).astype(BF)

        def scores(i, q, e):
            s = _dot_nt(q[:, e * T:(e + 1) * T], k_s[e, pl.ds(0, (i + 1) * T), :])
            sd = jnp.where(col <= row, s[:, i * T:], -1e9 * LOG2E)
            s = jnp.concatenate([s[:, :i * T], sd], axis=1) if i else sd
            return s, jnp.max(s, axis=1, keepdims=True)

        def context(i, s, m, e):
            pr = jnp.exp2(s - m)
            l = jnp.sum(pr, axis=1, keepdims=True)
            o = _dot(pr.astype(BF), v_s[e, pl.ds(0, (i + 1) * T), :])
            ctx_s[2 * p + e, pl.ds(i * T, T), :] = (o * (1.0 / l)).astype(BF)

        order = list(range(NB - 1, -1, -1))
        qs, ss = {}, {}
        for t in range(NB + 2):
            if t < NB:
                qs[t] = q_proj(order[t])
            for e in range(2):
                if 0 <= t - 1 < NB:
                    ss[t - 1, e] = scores(order[t - 1], qs[t - 1], e)
                if 0 <= t - 2 < NB:
                    context(order[t - 2], *ss.pop((t - 2, e)), e)
        return carry

    lax.fori_loop(0, NP, pair_body, 0)

    for cp in b_cp:
        cp.wait()

    def out_copy(j):
        return pltpu.make_async_copy(
            o_v.at[j], o_hbm.at[:, pl.ds(pl.multiple_of(j * T, T), T)], sem_o.at[j])

    def chan_body(j, carry):
        RC = 256
        NR = S // RC

        def a_proj(r):
            ctx = jnp.concatenate([ctx_s[h, pl.ds(r * RC, RC), :] for h in range(H)], axis=1)
            return _dot(ctx, wo_v[j])

        par = par_s[j]
        kpad[pl.ds(8, S), :] = bk_v[j].astype(F32)
        ksh = kpad[pl.ds(8, S), :] * par[0:1, :]
        for t in range(1, KS):
            ksh = ksh + kpad[pl.ds(8 - t, S), :] * par[t:t + 1, :]
        kv = ksh * bv_v[j].astype(F32)
        kvb = kv.astype(BF)

        fwd = fwd_ref[...]
        hb = h_v[pl.ds(pl.multiple_of(j * T, T), T), :]
        hf = _dot_nt(fwd, jnp.concatenate(
            [hb[:, a * T:(a + 1) * T] for a in range(NB)], axis=0))
        xf = _dot(fwd, jnp.concatenate(
            [kvb[a * T:(a + 1) * T, :] for a in range(NB)], axis=1))

        a_out = [a_proj(r) for r in range(NR - 1)]

        zr, zi = [], []
        for g in range(T // 8):
            def pick(v, off):
                return [v[off + g * 8:off + g * 8 + 8, a * T:(a + 1) * T] for a in range(NB)]
            xr, xi, hr0, hi0 = pick(xf, 0), pick(xf, T), pick(hf, 0), pick(hf, T)
            if g < T // 16:
                hr = [hr0[0]] + [hr0[m] - hi0[m - 1] for m in range(1, NB)]
                hi = [hi0[0]] + [hi0[m] + hr0[m - 1] for m in range(1, NB)]
            else:
                hr = [hr0[0]] + [hr0[m] + hi0[m - 1] for m in range(1, NB)]
                hi = [hi0[0]] + [hi0[m] - hr0[m - 1] for m in range(1, NB)]
            p1 = _causal_conv(xr, hr)
            p2 = _causal_conv(xi, hi)
            p3 = _causal_conv([u + v for u, v in zip(xr, xi)], [u + v for u, v in zip(hr, hi)])
            zr.append(jnp.concatenate([u - v for u, v in zip(p1, p2)], axis=1))
            zi.append(jnp.concatenate([w - u - v for u, v, w in zip(p1, p2, p3)], axis=1))
        z = jnp.concatenate(zr + zi, axis=0).astype(BF)
        y = _dot(inv_ref[...], z)
        a_out.append(a_proj(NR - 1))

        for a in range(NB):
            rows = pl.ds(a * T, T)
            ya = y[:, a * T:(a + 1) * T] + kv[a * T:(a + 1) * T, :] * par[KS:KS + 1, :]
            b = x_v[j, rows, :].astype(F32) * ya
            off = (a * T) % RC
            av = a_out[(a * T) // RC][off:off + T, :]
            g = g_s[rows, :]
            o_v[j, rows, :] = (g * av + (1.0 - g) * b).astype(BF)
        out_copy(j).start()
        return carry

    lax.fori_loop(0, NX, chan_body, 0)
    for j in range(NX):
        out_copy(j).wait()


@jax.jit
def pallas_gated_mix__compressed_kv_cla__ssm_conv_h3__prompt_kernel(
    A_x: jax.Array,
    A_c_kv: jax.Array,
    A_w_q: jax.Array,
    A_w_uk: jax.Array,
    A_w_uv: jax.Array,
    A_w_o: jax.Array,
    B_q: jax.Array,
    B_k: jax.Array,
    B_v: jax.Array,
    B_shift_k: jax.Array,
    B_ssm_k: jax.Array,
    B_ssm_D: jax.Array,
    gate_w: jax.Array,
):
    del B_q
    B, S, M = A_x.shape
    Dc, H, D = A_w_uk.shape
    assert B == 1 and D == T and A_c_kv.shape[1] == S
    NX, NC = M // T, Dc // T
    fwd, inv = _dft_matrices()

    vmem = pl.BlockSpec(memory_space=pltpu.VMEM)
    hbm = pl.BlockSpec(memory_space=pl.ANY)
    out = pl.pallas_call(
        _kernel,
        in_specs=[vmem] * 5 + [hbm] * 9,
        out_specs=hbm,
        out_shape=jax.ShapeDtypeStruct((S, M), BF),
        scratch_shapes=[
            pltpu.VMEM((NX, S, T), BF),
            pltpu.VMEM((NC, S, T), BF),
            pltpu.VMEM((2, M, T), jnp.uint32),
            pltpu.VMEM((2, Dc, T), jnp.uint32),
            pltpu.VMEM((2, Dc, T), jnp.uint32),
            pltpu.VMEM((M, 2 * T), BF),
            pltpu.VMEM((Dc, 4 * T), BF),
            pltpu.VMEM((2, S, T), BF),
            pltpu.VMEM((2, S, T), BF),
            pltpu.VMEM((H, S, T), BF),
            pltpu.VMEM((NX, H * D, T), BF),
            pltpu.VMEM((NX, S, T), BF),
            pltpu.VMEM((NX, S, T), BF),
            pltpu.VMEM((M, S), BF),
            pltpu.VMEM((S, T), F32),
            pltpu.VMEM((NX, 8, T), F32),
            pltpu.VMEM((S + 8, T), F32),
            pltpu.VMEM((NX, S, T), BF),
            pltpu.SemaphoreType.DMA,
            pltpu.SemaphoreType.DMA,
            pltpu.SemaphoreType.DMA((2, 3)),
            pltpu.SemaphoreType.DMA((4,)),
            pltpu.SemaphoreType.DMA((NX,)),
        ],
        compiler_params=pltpu.CompilerParams(vmem_limit_bytes=110 * 2**20),
        name="gated_mix_cla_h3",
    )(
        B_shift_k.T, B_ssm_D.reshape(NX, T), gate_w.reshape(NX, T), fwd, inv,
        A_x.reshape(S, M), A_c_kv.reshape(S, Dc), A_w_q, A_w_uk, A_w_uv,
        A_w_o.reshape(H * D, M), B_k.reshape(S, M), B_v.reshape(S, M), B_ssm_k,
    )
    return out.reshape(B, S, M)
```

```python
import numpy as np
import jax
import jax.numpy as jnp
from jax import lax
import jax.experimental.pallas as pl
import jax.experimental.pallas.tpu as pltpu

BF = jnp.bfloat16
F32 = jnp.float32
U32 = jnp.uint32
T = 128
P = T // 2
LOG2E = 1.4426950408889634


def _dft_matrices():
    w = np.pi * (2 * np.arange(T) + 0.5) / T
    fwd = w[:, None] * np.arange(T)[None, :]
    b = np.concatenate([np.arange(0, T, 2), np.arange(1, T, 2)])
    inv = b[:, None] * w[None, :P]
    return np.stack([np.cos(fwd), np.sin(fwd),
                     np.concatenate([np.cos(inv), np.sin(inv)], axis=1) / T]).astype(BF)


def _dot(a, b):
    return jnp.dot(a, b, preferred_element_type=F32)


def _dot_nt(a, b):
    return lax.dot_general(a, b, (((1,), (1,)), ((), ())), preferred_element_type=F32)


def _cat(xs, axis):
    return jnp.concatenate(xs, axis=axis) if len(xs) > 1 else xs[0]


def _bf(words):
    return pltpu.bitcast(words, BF)


def _f32(words):
    return _bf(words).astype(F32)


def _split_pair(words):
    return (pltpu.bitcast(words << 16, F32),
            pltpu.bitcast(words & np.uint32(0xFFFF0000), F32))


def _after(val, dep):
    dep = pltpu.bitcast(dep, F32)
    return jnp.where(dep < -jnp.inf, pltpu.bitcast(dep, val.dtype), val)


class _Pins:
    def __init__(self):
        self.clock = 0
        self.queue = []

    def add(self, dep, delay=0):
        self.queue.append((self.clock + delay, dep))
        self.queue.sort(key=lambda item: item[0])

    def tile(self, words):
        if self.queue and self.queue[0][0] <= self.clock:
            words = _after(words, self.queue.pop(0)[1])
        self.clock += 1
        return words


def _lhs_terms(a11, a12, a21, a22):
    return [a11 + a22, a21 + a22, a11, a22, a11 + a12, a21 - a11, a12 - a22]


def _rhs_terms(b11, b12, b21, b22):
    return [b11 + b22, b11, b12 - b22, b21 - b11, b22, b11 + b12, b21 + b22]


_SUM_SLOT = {0: 0, 1: 1, 4: 2, 5: 3, 6: 4}


def _strassen(lhs, rhs):
    m5, m3, m6, m1, m2, m4, m7 = [_dot(_bf(lhs(k)), _bf(rhs(k))) for k in (4, 2, 5, 0, 1, 3, 6)]
    return m1 - m5 + m4 + m7, m3 + m5, m2 + m4, m3 + m6 + m1 - m2


def _causal_conv(xs, hs):
    out = []
    for a in range(len(xs)):
        acc = xs[a] * hs[0]
        for m in range(1, a + 1):
            acc = acc + xs[a - m] * hs[m]
        out.append(acc)
    return out


def _kernel(x_hbm, c_hbm, wq_hbm, wk_hbm, wv_hbm, wo_hbm, bk_hbm, bv_hbm, h_hbm, dft_hbm,
            shift_hbm, d_hbm, gw_hbm,
            o_hbm,
            x_v, c_v, wq_v, wkv_v, wo_v, bk_v, bv_v, h_v, dft_v,
            xs_b, cs_b, wq_b, we_b, wd_b, wo_b, kv_b, ctx_b, u_b,
            xf_s, hf_s, y_s, g_s, par_s, o_v, shift_v, d_v, gw_v,
            sem_c, sem_0, sem_1, sem_2, sem_o):
    NU, _, _, M = x_v.shape
    NB = 2 * NU
    NX = M // T
    NP = kv_b.shape[0]
    NR = cs_b.shape[2]
    KS = shift_v.shape[0]
    qscale = (T ** -0.5) * LOG2E
    (x_hbm, c_hbm, wq_hbm, wk_hbm, wv_hbm, wo_hbm, bk_hbm, bv_hbm, h_hbm, dft_hbm) = (
        r.bitcast(U32) for r in
        (x_hbm, c_hbm, wq_hbm, wk_hbm, wv_hbm, wo_hbm, bk_hbm, bv_hbm, h_hbm, dft_hbm))
    xs_w, cs_w, wq_w, we_w, wd_w, wo_w, kv_w, ctx_w, u_w = (
        r.bitcast(U32) for r in (xs_b, cs_b, wq_b, we_b, wd_b, wo_b, kv_b, ctx_b, u_b))

    def blk(i, n=T):
        return pl.ds(i * n if isinstance(i, int) else pl.multiple_of(i * n, n), n)

    def c_copy(u):
        return pltpu.make_async_copy(c_hbm.at[u], c_v.at[u], sem_c.at[u])

    def wkv_copies(pair, slot, n):
        return [pltpu.make_async_copy(hbm.at[:, pair, :], wkv_v.at[slot, n, e], sem_1.at[slot])
                for e, hbm in enumerate((wk_hbm, wv_hbm))]

    def copies1(j, slot):
        sem = sem_1.at[slot]
        return ([pltpu.make_async_copy(h_hbm.at[j], h_v.at[slot], sem),
                 pltpu.make_async_copy(bk_hbm.at[:, blk(j)], bk_v.at[slot], sem),
                 pltpu.make_async_copy(bv_hbm.at[:, blk(j)], bv_v.at[slot], sem),
                 pltpu.make_async_copy(x_hbm.at[j], x_v.at[j], sem)]
                + wkv_copies(2 * j, slot, 0) + wkv_copies(2 * j + 1, slot, 1))

    def wq_copy(pair, slot):
        return pltpu.make_async_copy(wq_hbm.at[:, pair, :], wq_v.at[slot], sem_2.at[slot])

    def copies2(p, slot):
        return [wq_copy((p + 1) & (NP - 1), slot),
                pltpu.make_async_copy(wo_hbm.at[blk(p, 2)], wo_v.at[slot], sem_2.at[slot])]

    def out_copy(u, n):
        at = (u, slice(None), slice(None), blk(n, 2 * T))
        return pltpu.make_async_copy(o_v.at[at], o_hbm.at[at], sem_o)

    def lhs_operands(src, dst, u):
        half = dst.shape[2]
        for n in range(half):
            q = [_f32(src[u, a, :, blk(n + b * half)]) for a in (0, 1) for b in (0, 1)]
            for k, t in enumerate(_lhs_terms(*q)):
                if k in _SUM_SLOT:
                    dst[_SUM_SLOT[k], u, n] = t.astype(BF)

    def lhs_loader(src, sums, u, pins):
        half = sums.shape[2]

        def lhs(k):
            if k in _SUM_SLOT:
                tiles = [sums[_SUM_SLOT[k], u, n] for n in range(half)]
            else:
                tiles = [src[u, k - 2, :, blk(n + (k - 2) * half)] for n in range(half)]
            return _cat([pins.tile(t) for t in tiles], 1)
        return lhs

    def rhs_operands(src, dst, *at):
        half = dst.shape[-3]
        for n in range(half):
            b11, b12 = _split_pair(src[blk(n), :])
            b21, b22 = _split_pair(src[blk(n + half), :])
            for k, t in enumerate(_rhs_terms(b11, b12, b21, b22)):
                dst[(*at, k, n)] = t.astype(BF)

    def kv_proj(pair, u, w, slot, pins, start=()):
        c = _strassen(lhs_loader(c_v, cs_w, u, pins),
                      lambda k: _cat([_cat([w[slot, e, k, r] for r in range(NR)], 0)
                                      for e in (0, 1)], 1))
        for cp in start:
            cp.start()
        for a in (0, 1):
            for b in (0, 1):
                for e in (0, 1):
                    kv_b[pair, u, 4 * e + 2 * b + a] = c[2 * a + b][:, e * T:(e + 1) * T].astype(BF)

    small = [pltpu.make_async_copy(s, d, sem_0) for s, d in
             ((dft_hbm, dft_v), (shift_hbm, shift_v), (d_hbm, d_v), (gw_hbm, gw_v))]
    for cp in (wkv_copies(NP - 1, 1, 0) + [c_copy(u) for u in range(NU)]
               + small + copies1(0, 0) + [wq_copy(0, 1)] + copies2(0, 0)):
        cp.start()
    for cp in wkv_copies(NP - 1, 1, 0):
        cp.wait()
    for e in (0, 1):
        rhs_operands(wkv_v.at[1, 0, e], we_b, 0, e)

    def stage0(u, carry):
        c_copy(u).wait()
        lhs_operands(c_v, cs_b, u)
        kv_proj(NP - 1, u, we_w, 0, _Pins())
        return carry

    lax.fori_loop(0, NU, stage0, 0)

    for cp in small:
        cp.wait()
    shift = shift_v[...].astype(F32)
    dvec = d_v[...].astype(F32)
    for j in range(NX):
        par_s[j, 0:KS, :] = shift[:, j * T:(j + 1) * T]
        par_s[j, KS:KS + 1, :] = dvec[j:j + 1, :]

    def stage1(j, carry):
        slot = j & 1
        zero = j >> 16
        pins = _Pins()
        for cp in copies1(j, slot):
            cp.wait()

        def step(t):
            if t < NU:
                start = copies1((j + 1) & (NX - 1), 1 - slot) if t == 3 else ()
                kv_proj(2 * j, t, we_w, 0, pins, start)
            else:
                new = (t - NU >= j).astype(jnp.int32)
                kv_proj(2 * (j + new) - 1, t - NU + new, wd_w, slot ^ new ^ 1, pins)

        def w_operands(n, dst, words, at, delay, stride):
            for e in (0, 1):
                rhs_operands(wkv_v.at[slot, n, e], dst, at, e)
                for r in range(NR):
                    dep = pltpu.bitcast(words[at, e, 0, r], F32)
                    for k in range(1, 7):
                        dep = jnp.maximum(dep, pltpu.bitcast(words[at, e, k, r], F32))
                    pins.add(dep, delay + stride * (NR * e + r))

        def forward(dst, dot, tiles):
            for a in range(0, NB, 4):
                fwd = _bf(_cat([pins.tile(dft_v[0]), pins.tile(dft_v[1])], 0))
                dst[zero, :, blk(a // 4, 4 * T)] = dot(fwd, tiles(a))

        w_operands(0, we_b, we_w, 0, 2, 1)
        forward(hf_s, _dot_nt,
                lambda a: _bf(_cat([h_v[slot, :, blk(a + n)] for n in range(4)], 0)))

        prev = jnp.zeros((8, T), F32)
        for a in range(NB):
            cur = _f32(bk_v[slot, blk(a, P), :])
            ext = _cat([prev, cur], 0)
            prev = cur[T - 8:]
            ksh = cur * par_s[j, 0:1, :]
            for t in range(1, KS):
                ksh = ksh + pltpu.roll(ext, t, 0)[8:] * par_s[j, t:t + 1, :]
            kv = ksh * _f32(bv_v[slot, blk(a, P), :])
            y_s[j, a, 0:T, :] = kv * par_s[j, KS:KS + 1, :]
            u_b[a] = kv.astype(BF)
            pins.add(u_w[a], 2 + 2 * a)
        for t in range(3):
            step(t)
        forward(xf_s, _dot, lambda a: _bf(_cat([u_w[a + n] for n in range(4)], 1)))
        step(3)
        w_operands(1, wd_b, wd_w, slot, 6, 6)

        def pin(vals, at):
            at = 2 * (13 * at // 10)
            pins.add(_cat(vals[0::2], 0), at)
            pins.add(_cat(vals[1::2], 0), at)
            return vals

        def spectrum(g, at):
            def pick(ref, off):
                return [ref[0, pl.ds(off + g * 8, 8), blk(a)] for a in range(NB)]
            xr, xi, hr, hi = pick(xf_s, 0), pick(xf_s, T), pick(hf_s, 0), pick(hf_s, T)
            hr, hi = ([hr[0]] + [hr[m] + hi[m - 1] for m in range(1, NB)],
                      [hi[0]] + [hi[m] - hr[m - 1] for m in range(1, NB)])
            p1 = pin(_causal_conv(xr, hr), at)
            p2 = _causal_conv(xi, hi)
            zr = pin([u - v for u, v in zip(p1, p2)], at + 1)
            p3 = _causal_conv([u + v for u, v in zip(xr, xi)], [u + v for u, v in zip(hr, hi)])
            zi = pin([w - (u + v) for u, v, w in zip(p1, p2, p3)], at + 2)
            return _cat(zr, 1), _cat(zi, 1)

        z = [(spectrum(g, 6 * g), spectrum(g + P // 8, 6 * g + 3)) for g in range(P // 8)]
        for t in range(4, 2 * NU - 3):
            step(t)

        lhs_operands(x_v, xs_b, j)
        for n in range(NX // 2):
            for k in range(5):
                pins.add(xs_w[k, j, n])
        gw = gw_v[...].astype(F32)
        for a in (0, 1):
            acc = _f32(x_v[j, a, :, blk(0)]) * gw[0:1, :]
            for n in range(1, NX):
                acc = acc + _f32(x_v[j, a, :, blk(n)]) * gw[n:n + 1, :]
            g = jnp.broadcast_to(jax.nn.sigmoid(jnp.sum(acc, axis=1, keepdims=True)), (T, T))
            g_s[j, a] = g
            pins.add(jnp.maximum(g[:P], g[P:]), 22 + 4 * a)
        step(2 * NU - 3)
        step(2 * NU - 2)
        for odd in (0, 1):
            zz = [u[c] - v[c] if odd else u[c] + v[c] for c in (0, 1) for u, v in z]
            y = _dot(_bf(dft_v[2, blk(odd, P // 2), :]), _cat(zz, 0).astype(BF))
            for a in range(NB):
                y_s[j, a, pl.ds(odd, P, stride=2), :] += y[:, a * T:(a + 1) * T]
        return carry

    lax.fori_loop(0, NX, stage1, 0)

    for cp in copies1(0, 0):
        cp.wait()
    wq_copy(0, 1).wait()
    rhs_operands(wq_v.at[1], wq_b)

    def stage2(p, carry):
        slot = p & 1
        pins = _Pins()
        for cp in copies2(p, slot):
            cp.wait()
        row = lax.broadcasted_iota(jnp.int32, (T, T), 0)
        col = lax.broadcasted_iota(jnp.int32, (T, T), 1)
        qs, ss, cc = {}, {}, {}

        def q_proj(u):
            c = _strassen(lhs_loader(x_v, xs_w, u, pins),
                          lambda k: _cat([wq_w[k, r] for r in range(NX // 2)], 0))
            for a in (0, 1):
                for b in (0, 1):
                    qs[2 * u + a, b] = c[2 * a + b] * qscale

        def keys_or_values(which, e, i):
            return _bf(_cat([kv_w[p, n // 2, 4 * which + 2 * e + n % 2] for n in range(i + 1)], 0))

        def scores(i, e, q):
            s = _dot_nt(q.astype(BF), keys_or_values(0, e, i))
            sd = jnp.where(col <= row, s[:, i * T:], -1e9 * LOG2E)
            s = _cat([s[:, :i * T], sd], 1) if i else sd
            return s, jnp.max(s, axis=1, keepdims=True)

        def context(i, e, s, m):
            pr = jnp.exp2(s - m).astype(BF)
            l = jnp.sum(pr.astype(F32), axis=1, keepdims=True)
            r = pl.reciprocal(l, approx=True)
            r = r * (2.0 - l * r)
            return _dot(pr, keys_or_values(1, e, i)) * r

        order = [2 * u + a for u in (5, 6, 0, 7, 2, 4, 3, 1) for a in (1, 0)]
        q_proj(order[0] // 2)
        for cp in copies2((p + 1) & (NP - 1), 1 - slot):
            cp.start()
        for n in range(NX // 2):
            w = [_f32(wo_v[slot, a, :, blk(2 * n + b)]) for a in (0, 1) for b in (0, 1)]
            for k, v in enumerate(_rhs_terms(*w)):
                wo_b[k, n, p] = v.astype(BF)
                pins.add(wo_w[k, n, p])
        for t in range(NB + 1):
            if t % 2 == 0 and t + 2 < NB:
                q_proj(order[t + 2] // 2)
            if t + 4 == NB:
                rhs_operands(wq_v.at[slot], wq_b)
            for e in (0, 1):
                if t < NB:
                    q = qs.pop((order[t], e))
                    if t >= 3:
                        q = _after(q, cc[order[t - 3], e])
                    ss[t, e] = scores(order[t], e, q)
                if t >= 1:
                    cc[order[t - 1], e] = context(order[t - 1], e, *ss.pop((t - 1, e)))
            if t >= 2 and t % 2 == 0:
                u = order[t - 1] // 2
                terms = _lhs_terms(cc[2 * u, 0], cc[2 * u, 1], cc[2 * u + 1, 0], cc[2 * u + 1, 1])
                for k, v in enumerate(terms):
                    ctx_b[k, u, p] = v.astype(BF)
                    pins.add(ctx_w[k, u, p], 4 + 2 * k)
        return carry

    lax.fori_loop(0, NP, stage2, 0)

    for cp in copies2(0, 0):
        cp.wait()

    def stage3(u, carry):
        for n in range(NX // 2):
            c = _strassen(lambda k: _cat([ctx_w[k, u, p] for p in range(NP)], 1),
                          lambda k: _cat([wo_w[k, n, p] for p in range(NP)], 0))
            if n:
                out_copy(u, n - 1).start()
            for a in (0, 1):
                g = g_s[u, a]
                for b in (0, 1):
                    j = 2 * n + b
                    bb = _f32(x_v[u, a, :, blk(j)]) * y_s[j, 2 * u + a, 0:T, :]
                    o_v[u, a, :, blk(j)] = (g * c[2 * a + b] + (1.0 - g) * bb).astype(BF)
        out_copy(u, NX // 2 - 1).start()
        return carry

    lax.fori_loop(0, NU, stage3, 0)
    for u in range(NU):
        for n in range(NX // 2):
            out_copy(u, n).wait()


@jax.jit
def pallas_gated_mix__compressed_kv_cla__ssm_conv_h3__prompt_kernel(
    A_x: jax.Array,
    A_c_kv: jax.Array,
    A_w_q: jax.Array,
    A_w_uk: jax.Array,
    A_w_uv: jax.Array,
    A_w_o: jax.Array,
    B_q: jax.Array,
    B_k: jax.Array,
    B_v: jax.Array,
    B_shift_k: jax.Array,
    B_ssm_k: jax.Array,
    B_ssm_D: jax.Array,
    gate_w: jax.Array,
):
    del B_q
    B, S, M = A_x.shape
    Dc, H, D = A_w_uk.shape
    KS = B_shift_k.shape[1]
    NX, NB, NP = M // T, S // T, H // 2
    NU = NB // 2
    assert B == 1 and D == T and A_c_kv.shape[1] == S
    assert NU == NX == 8 and NP == 2 * NX and KS < 8

    hbm = pl.BlockSpec(memory_space=pl.ANY)
    out = pl.pallas_call(
        _kernel,
        in_specs=[hbm] * 13,
        out_specs=hbm,
        out_shape=jax.ShapeDtypeStruct((NU, 2, T, M), BF),
        scratch_shapes=[
            pltpu.VMEM((NU, 2, P, M), U32),
            pltpu.VMEM((NU, 2, P, Dc), U32),
            pltpu.VMEM((2, M, T), U32),
            pltpu.VMEM((2, 2, 2, Dc, T), U32),
            pltpu.VMEM((2, 2, P, M), U32),
            pltpu.VMEM((2, S // 2, T), U32),
            pltpu.VMEM((2, S // 2, T), U32),
            pltpu.VMEM((2, P, S), U32),
            pltpu.VMEM((3, P, T), U32),
            pltpu.VMEM((5, NU, M // (2 * T), T, T), BF),
            pltpu.VMEM((5, NU, Dc // (2 * T), T, T), BF),
            pltpu.VMEM((7, M // (2 * T), T, T), BF),
            pltpu.VMEM((1, 2, 7, Dc // (2 * T), T, T), BF),
            pltpu.VMEM((2, 2, 7, Dc // (2 * T), T, T), BF),
            pltpu.VMEM((7, NX // 2, NP, T, T), BF),
            pltpu.VMEM((NP, NU, 8, T, T), BF),
            pltpu.VMEM((7, NU, NP, T, T), BF),
            pltpu.VMEM((NB, T, T), BF),
            pltpu.VMEM((1, 2 * T, S), F32),
            pltpu.VMEM((1, 2 * T, S), F32),
            pltpu.VMEM((NX, NB, T + 8, T), F32),
            pltpu.VMEM((NU, 2, T, T), F32),
            pltpu.VMEM((NX, 8, T), F32),
            pltpu.VMEM((NU, 2, T, M), BF),
            pltpu.VMEM((KS, M), BF),
            pltpu.VMEM((NX, T), BF),
            pltpu.VMEM((NX, T), BF),
            pltpu.SemaphoreType.DMA((NU,)),
            pltpu.SemaphoreType.DMA,
            pltpu.SemaphoreType.DMA((2,)),
            pltpu.SemaphoreType.DMA((2,)),
            pltpu.SemaphoreType.DMA,
        ],
        compiler_params=pltpu.CompilerParams(vmem_limit_bytes=124 * 2**20),
        name="gated_mix_cla_h3",
    )(
        A_x.reshape(NU, 2, T, M), A_c_kv.reshape(NU, 2, T, Dc), A_w_q, A_w_uk, A_w_uv,
        A_w_o, B_k.reshape(S, M), B_v.reshape(S, M), B_ssm_k.reshape(NX, T, S),
        _dft_matrices(), B_shift_k.T, B_ssm_D.reshape(NX, T), gate_w.reshape(NX, T),
    )
    return out.reshape(B, S, M)
```

```python
import numpy as np
import jax
import jax.numpy as jnp
from jax import lax
import jax.experimental.pallas as pl
import jax.experimental.pallas.tpu as pltpu

BF = jnp.bfloat16
F32 = jnp.float32
U32 = jnp.uint32
T = 128
P = T // 2
LOG2E = 1.4426950408889634


def _dft_matrices():
    w = np.pi * (2 * np.arange(T) + 0.5) / T
    fwd = w[:, None] * np.arange(T)[None, :]
    b = np.concatenate([np.arange(0, T, 2), np.arange(1, T, 2)])
    inv = b[:, None] * w[None, :P]
    return np.stack([np.cos(fwd), np.sin(fwd),
                     np.concatenate([np.cos(inv), np.sin(inv)], axis=1) / T]).astype(BF)


def _dot(a, b):
    return jnp.dot(a, b, preferred_element_type=F32)


def _dot_nt(a, b):
    return lax.dot_general(a, b, (((1,), (1,)), ((), ())), preferred_element_type=F32)


def _cat(xs, axis):
    return jnp.concatenate(xs, axis=axis) if len(xs) > 1 else xs[0]


def _bf(words):
    return pltpu.bitcast(words, BF)


def _f32(words):
    return _bf(words).astype(F32)


def _split_pair(words):
    return (pltpu.bitcast(words << 16, F32),
            pltpu.bitcast(words & np.uint32(0xFFFF0000), F32))


def _after(val, dep):
    dep = pltpu.bitcast(dep, F32)
    return jnp.where(dep < -jnp.inf, pltpu.bitcast(dep, val.dtype), val)


class _Pins:
    def __init__(self):
        self.clock = 0
        self.queue = []

    def add(self, dep, delay=0):
        self.queue.append((self.clock + delay, dep))
        self.queue.sort(key=lambda item: item[0])

    def tile(self, words):
        if self.queue and self.queue[0][0] <= self.clock:
            words = _after(words, self.queue.pop(0)[1])
        self.clock += 1
        return words


def _lhs_terms(a11, a12, a21, a22):
    return [a11 + a22, a21 + a22, a11, a22, a11 + a12, a21 - a11, a12 - a22]


def _rhs_terms(b11, b12, b21, b22):
    return [b11 + b22, b11, b12 - b22, b21 - b11, b22, b11 + b12, b21 + b22]


_SUM_SLOT = {0: 0, 1: 1, 4: 2, 5: 3, 6: 4}


def _strassen(lhs, rhs):
    m5, m3, m6, m1, m2, m4, m7 = [_dot(_bf(lhs(k)), _bf(rhs(k))) for k in (4, 2, 5, 0, 1, 3, 6)]
    return m1 - m5 + m4 + m7, m3 + m5, m2 + m4, m3 + m6 + m1 - m2


def _causal_conv(xs, hs):
    out = []
    for a in range(len(xs)):
        acc = xs[a] * hs[0]
        for m in range(1, a + 1):
            acc = acc + xs[a - m] * hs[m]
        out.append(acc)
    return out


def _kernel(x_hbm, c_hbm, wq_hbm, wk_hbm, wv_hbm, wo_hbm, bk_hbm, bv_hbm, h_hbm, dft_hbm,
            shift_hbm, d_hbm, gw_hbm,
            o_hbm,
            x_v, c_v, wq_v, wkv_v, wo_v, bk_v, bv_v, h_v, dft_v,
            xs_b, cs_b, wq_b, we_b, wd_b, wo_b, kv_b, ctx_b, u_b,
            xf_s, hf_s, y_s, g_s, par_s, o_v, shift_v, d_v, gw_v,
            sem_c, sem_0, sem_1, sem_2, sem_o):
    NU, _, _, M = x_v.shape
    NB = 2 * NU
    NX = M // T
    NP = kv_b.shape[0]
    NR = cs_b.shape[2]
    KS = shift_v.shape[0]
    qscale = (T ** -0.5) * LOG2E
    (x_hbm, c_hbm, wq_hbm, wk_hbm, wv_hbm, wo_hbm, bk_hbm, bv_hbm, h_hbm, dft_hbm) = (
        r.bitcast(U32) for r in
        (x_hbm, c_hbm, wq_hbm, wk_hbm, wv_hbm, wo_hbm, bk_hbm, bv_hbm, h_hbm, dft_hbm))
    xs_w, cs_w, wq_w, we_w, wd_w, wo_w, kv_w, ctx_w, u_w = (
        r.bitcast(U32) for r in (xs_b, cs_b, wq_b, we_b, wd_b, wo_b, kv_b, ctx_b, u_b))

    def blk(i, n=T):
        return pl.ds(i * n if isinstance(i, int) else pl.multiple_of(i * n, n), n)

    def c_copy(u):
        return pltpu.make_async_copy(c_hbm.at[u], c_v.at[u], sem_c.at[u])

    def wkv_copies(pair, slot, n):
        return [pltpu.make_async_copy(hbm.at[:, pair, :], wkv_v.at[slot, n, e], sem_1.at[slot])
                for e, hbm in enumerate((wk_hbm, wv_hbm))]

    def copies1(j, slot):
        sem = sem_1.at[slot]
        return (wkv_copies(2 * j, slot, 0) + wkv_copies(2 * j + 1, slot, 1)
                + [pltpu.make_async_copy(bk_hbm.at[:, blk(j)], bk_v.at[slot], sem),
                   pltpu.make_async_copy(bv_hbm.at[:, blk(j)], bv_v.at[slot], sem),
                   pltpu.make_async_copy(h_hbm.at[j], h_v.at[slot], sem),
                   pltpu.make_async_copy(x_hbm.at[j], x_v.at[j], sem)])

    def wq_copy(pair, slot):
        return pltpu.make_async_copy(wq_hbm.at[:, pair, :], wq_v.at[slot], sem_2.at[slot])

    def copies2(p, slot):
        return [wq_copy((p + 1) & (NP - 1), slot),
                pltpu.make_async_copy(wo_hbm.at[blk(p, 2)], wo_v.at[slot], sem_2.at[slot])]

    def out_copy(u, n):
        at = (u, slice(None), slice(None), blk(n, 2 * T))
        return pltpu.make_async_copy(o_v.at[at], o_hbm.at[at], sem_o)

    def lhs_operands(src, dst, u):
        half = dst.shape[2]
        for n in range(half):
            q = [_f32(src[u, a, :, blk(n + b * half)]) for a in (0, 1) for b in (0, 1)]
            for k, t in enumerate(_lhs_terms(*q)):
                if k in _SUM_SLOT:
                    dst[_SUM_SLOT[k], u, n] = t.astype(BF)

    def lhs_loader(src, sums, u, pins):
        half = sums.shape[2]

        def lhs(k):
            if k in _SUM_SLOT:
                tiles = [sums[_SUM_SLOT[k], u, n] for n in range(half)]
            else:
                tiles = [src[u, k - 2, :, blk(n + (k - 2) * half)] for n in range(half)]
            return _cat([pins.tile(t) for t in tiles], 1)
        return lhs

    def rhs_operands(src, dst, *at):
        half = dst.shape[-3]
        for n in range(half):
            b11, b12 = _split_pair(src[blk(n), :])
            b21, b22 = _split_pair(src[blk(n + half), :])
            for k, t in enumerate(_rhs_terms(b11, b12, b21, b22)):
                dst[(*at, k, n)] = t.astype(BF)

    def kv_proj(pair, u, w, slot, pins, start=()):
        c = _strassen(lhs_loader(c_v, cs_w, u, pins),
                      lambda k: _cat([_cat([w[slot, e, k, r] for r in range(NR)], 0)
                                      for e in (0, 1)], 1))
        for cp in start:
            cp.start()
        for a in (0, 1):
            for b in (0, 1):
                for e in (0, 1):
                    kv_b[pair, u, 4 * e + 2 * b + a] = c[2 * a + b][:, e * T:(e + 1) * T].astype(BF)

    small = [pltpu.make_async_copy(s, d, sem_0) for s, d in
             ((dft_hbm, dft_v), (shift_hbm, shift_v), (d_hbm, d_v), (gw_hbm, gw_v))]
    for cp in wkv_copies(NP - 1, 1, 0) + [c_copy(u) for u in range(NU)] + small + copies1(0, 0):
        cp.start()
    for cp in wkv_copies(NP - 1, 1, 0):
        cp.wait()
    for e in (0, 1):
        rhs_operands(wkv_v.at[1, 0, e], we_b, 0, e)

    def stage0(u, carry):
        c_copy(u).wait()
        lhs_operands(c_v, cs_b, u)
        kv_proj(NP - 1, u, we_w, 0, _Pins())
        return carry

    lax.fori_loop(0, NU, stage0, 0)

    for cp in [wq_copy(0, 1)] + copies2(0, 0):
        cp.start()
    for cp in small:
        cp.wait()
    shift = shift_v[...].astype(F32)
    dvec = d_v[...].astype(F32)
    for j in range(NX):
        par_s[j, 0:KS, :] = shift[:, j * T:(j + 1) * T]
        par_s[j, KS:KS + 1, :] = dvec[j:j + 1, :]

    def stage1(j, carry):
        slot = j & 1
        zero = j >> 16
        pins = _Pins()
        for cp in copies1(j, slot):
            cp.wait()

        def step(t):
            if t < NU:
                start = copies1((j + 1) & (NX - 1), 1 - slot) if t == 3 else ()
                kv_proj(2 * j, t, we_w, 0, pins, start)
            else:
                new = (t - NU >= j).astype(jnp.int32)
                kv_proj(2 * (j + new) - 1, t - NU + new, wd_w, slot ^ new ^ 1, pins)

        def w_operands(n, dst, words, at, delay, stride):
            for e in (0, 1):
                rhs_operands(wkv_v.at[slot, n, e], dst, at, e)
                for r in range(NR):
                    dep = pltpu.bitcast(words[at, e, 0, r], F32)
                    for k in range(1, 7):
                        dep = jnp.maximum(dep, pltpu.bitcast(words[at, e, k, r], F32))
                    pins.add(dep, delay + stride * (NR * e + r))

        def forward(dst, dot, tiles):
            for a in range(0, NB, 4):
                fwd = _bf(_cat([pins.tile(dft_v[0]), pins.tile(dft_v[1])], 0))
                dst[zero, :, blk(a // 4, 4 * T)] = dot(fwd, tiles(a))

        w_operands(0, we_b, we_w, 0, 2, 1)
        forward(hf_s, _dot_nt,
                lambda a: _bf(_cat([h_v[slot, :, blk(a + n)] for n in range(4)], 0)))

        prev = jnp.zeros((8, T), F32)
        for a in range(NB):
            cur = _f32(bk_v[slot, blk(a, P), :])
            ext = _cat([prev, cur], 0)
            prev = cur[T - 8:]
            ksh = cur * par_s[j, 0:1, :]
            for t in range(1, KS):
                ksh = ksh + pltpu.roll(ext, t, 0)[8:] * par_s[j, t:t + 1, :]
            kv = ksh * _f32(bv_v[slot, blk(a, P), :])
            y_s[j, a, 0:T, :] = kv * par_s[j, KS:KS + 1, :]
            u_b[a] = kv.astype(BF)
            pins.add(u_w[a], 2 + 2 * a)
        for t in range(3):
            step(t)
        forward(xf_s, _dot, lambda a: _bf(_cat([u_w[a + n] for n in range(4)], 1)))
        step(3)
        w_operands(1, wd_b, wd_w, slot, 6, 6)

        def pin(vals, at):
            at = 2 * (13 * at // 10)
            pins.add(_cat(vals[0::2], 0), at)
            pins.add(_cat(vals[1::2], 0), at)
            return vals

        def spectrum(g, at):
            def pick(ref, off):
                return [ref[0, pl.ds(off + g * 8, 8), blk(a)] for a in range(NB)]
            xr, xi, hr, hi = pick(xf_s, 0), pick(xf_s, T), pick(hf_s, 0), pick(hf_s, T)
            hr, hi = ([hr[0]] + [hr[m] + hi[m - 1] for m in range(1, NB)],
                      [hi[0]] + [hi[m] - hr[m - 1] for m in range(1, NB)])
            p1 = pin(_causal_conv(xr, hr), at)
            p2 = _causal_conv(xi, hi)
            zr = pin([u - v for u, v in zip(p1, p2)], at + 1)
            p3 = _causal_conv([u + v for u, v in zip(xr, xi)], [u + v for u, v in zip(hr, hi)])
            zi = pin([w - (u + v) for u, v, w in zip(p1, p2, p3)], at + 2)
            return _cat(zr, 1), _cat(zi, 1)

        z = [(spectrum(g, 6 * g), spectrum(g + P // 8, 6 * g + 3)) for g in range(P // 8)]
        for t in range(4, 2 * NU - 3):
            step(t)

        lhs_operands(x_v, xs_b, j)
        for n in range(NX // 2):
            for k in range(5):
                pins.add(xs_w[k, j, n])
        gw = gw_v[...].astype(F32)
        for a in (0, 1):
            acc = _f32(x_v[j, a, :, blk(0)]) * gw[0:1, :]
            for n in range(1, NX):
                acc = acc + _f32(x_v[j, a, :, blk(n)]) * gw[n:n + 1, :]
            g = jnp.broadcast_to(jax.nn.sigmoid(jnp.sum(acc, axis=1, keepdims=True)), (T, T))
            g_s[j, a] = g
            pins.add(jnp.maximum(g[:P], g[P:]), 22 + 4 * a)
        step(2 * NU - 3)
        step(2 * NU - 2)
        for odd in (0, 1):
            zz = [u[c] - v[c] if odd else u[c] + v[c] for c in (0, 1) for u, v in z]
            y = _dot(_bf(dft_v[2, blk(odd, P // 2), :]), _cat(zz, 0).astype(BF))
            for a in range(NB):
                y_s[j, a, pl.ds(odd, P, stride=2), :] += y[:, a * T:(a + 1) * T]
        return carry

    lax.fori_loop(0, NX, stage1, 0)

    for cp in copies1(0, 0):
        cp.wait()
    wq_copy(0, 1).wait()
    rhs_operands(wq_v.at[1], wq_b)

    def stage2(p, carry):
        slot = p & 1
        pins = _Pins()
        for cp in copies2(p, slot):
            cp.wait()
        row = lax.broadcasted_iota(jnp.int32, (T, T), 0)
        col = lax.broadcasted_iota(jnp.int32, (T, T), 1)
        qs, ss, cc = {}, {}, {}

        def q_proj(u):
            c = _strassen(lhs_loader(x_v, xs_w, u, pins),
                          lambda k: _cat([wq_w[k, r] for r in range(NX // 2)], 0))
            for a in (0, 1):
                for b in (0, 1):
                    qs[2 * u + a, b] = c[2 * a + b] * qscale

        def keys_or_values(which, e, i):
            return _bf(_cat([kv_w[p, n // 2, 4 * which + 2 * e + n % 2] for n in range(i + 1)], 0))

        def scores(i, e, q):
            s = _dot_nt(q.astype(BF), keys_or_values(0, e, i))
            sd = jnp.where(col <= row, s[:, i * T:], -1e9 * LOG2E)
            s = _cat([s[:, :i * T], sd], 1) if i else sd
            return s, jnp.max(s, axis=1, keepdims=True)

        def context(i, e, s, m):
            pr = jnp.exp2(s - m).astype(BF)
            l = jnp.sum(pr.astype(F32), axis=1, keepdims=True)
            r = pltpu.reciprocal(l, full_range=False)
            return _dot(pr, keys_or_values(1, e, i)) * r

        order = [2 * u + a for u in (5, 7, 0, 6, 2, 4, 3, 1) for a in (1, 0)]
        q_proj(order[0] // 2)
        for cp in copies2((p + 1) & (NP - 1), 1 - slot):
            cp.start()
        for n in range(NX // 2):
            w = [_f32(wo_v[slot, a, :, blk(2 * n + b)]) for a in (0, 1) for b in (0, 1)]
            for k, v in enumerate(_rhs_terms(*w)):
                wo_b[k, n, p] = v.astype(BF)
                pins.add(wo_w[k, n, p])
        for t in range(NB + 1):
            if t % 2 == 0 and t + 2 < NB:
                q_proj(order[t + 2] // 2)
            if t + 4 == NB:
                rhs_operands(wq_v.at[slot], wq_b)
            for e in (0, 1):
                if t < NB:
                    q = qs.pop((order[t], e))
                    if t >= 3:
                        q = _after(q, cc[order[t - 3], e])
                    ss[t, e] = scores(order[t], e, q)
                if t >= 1:
                    cc[order[t - 1], e] = context(order[t - 1], e, *ss.pop((t - 1, e)))
            if t >= 2 and t % 2 == 0:
                u = order[t - 1] // 2
                terms = _lhs_terms(cc[2 * u, 0], cc[2 * u, 1], cc[2 * u + 1, 0], cc[2 * u + 1, 1])
                for k, v in enumerate(terms):
                    ctx_b[k, u, p] = v.astype(BF)
                    pins.add(ctx_w[k, u, p], 8 + 2 * k)
        return carry

    lax.fori_loop(0, NP, stage2, 0)

    for cp in copies2(0, 0):
        cp.wait()

    def stage3(u, carry):
        for n in range(NX // 2):
            c = _strassen(lambda k: _cat([ctx_w[k, u, p] for p in range(NP)], 1),
                          lambda k: _cat([wo_w[k, n, p] for p in range(NP)], 0))
            if n:
                out_copy(u, n - 1).start()
            for a in (0, 1):
                g = g_s[u, a]
                for b in (0, 1):
                    j = 2 * n + b
                    bb = _f32(x_v[u, a, :, blk(j)]) * y_s[j, 2 * u + a, 0:T, :]
                    o_v[u, a, :, blk(j)] = (g * c[2 * a + b] + (1.0 - g) * bb).astype(BF)
        out_copy(u, NX // 2 - 1).start()
        return carry

    lax.fori_loop(0, NU, stage3, 0)
    for u in range(NU):
        for n in range(NX // 2):
            out_copy(u, n).wait()


@jax.jit
def pallas_gated_mix__compressed_kv_cla__ssm_conv_h3__prompt_kernel(
    A_x: jax.Array,
    A_c_kv: jax.Array,
    A_w_q: jax.Array,
    A_w_uk: jax.Array,
    A_w_uv: jax.Array,
    A_w_o: jax.Array,
    B_q: jax.Array,
    B_k: jax.Array,
    B_v: jax.Array,
    B_shift_k: jax.Array,
    B_ssm_k: jax.Array,
    B_ssm_D: jax.Array,
    gate_w: jax.Array,
):
    del B_q
    B, S, M = A_x.shape
    Dc, H, D = A_w_uk.shape
    KS = B_shift_k.shape[1]
    NX, NB, NP = M // T, S // T, H // 2
    NU = NB // 2
    assert B == 1 and D == T and A_c_kv.shape[1] == S
    assert NU == NX == 8 and NP == 2 * NX and KS < 8

    hbm = pl.BlockSpec(memory_space=pl.ANY)
    out = pl.pallas_call(
        _kernel,
        in_specs=[hbm] * 13,
        out_specs=hbm,
        out_shape=jax.ShapeDtypeStruct((NU, 2, T, M), BF),
        scratch_shapes=[
            pltpu.VMEM((NU, 2, P, M), U32),
            pltpu.VMEM((NU, 2, P, Dc), U32),
            pltpu.VMEM((2, M, T), U32),
            pltpu.VMEM((2, 2, 2, Dc, T), U32),
            pltpu.VMEM((2, 2, P, M), U32),
            pltpu.VMEM((2, S // 2, T), U32),
            pltpu.VMEM((2, S // 2, T), U32),
            pltpu.VMEM((2, P, S), U32),
            pltpu.VMEM((3, P, T), U32),
            pltpu.VMEM((5, NU, M // (2 * T), T, T), BF),
            pltpu.VMEM((5, NU, Dc // (2 * T), T, T), BF),
            pltpu.VMEM((7, M // (2 * T), T, T), BF),
            pltpu.VMEM((1, 2, 7, Dc // (2 * T), T, T), BF),
            pltpu.VMEM((2, 2, 7, Dc // (2 * T), T, T), BF),
            pltpu.VMEM((7, NX // 2, NP, T, T), BF),
            pltpu.VMEM((NP, NU, 8, T, T), BF),
            pltpu.VMEM((7, NU, NP, T, T), BF),
            pltpu.VMEM((NB, T, T), BF),
            pltpu.VMEM((1, 2 * T, S), F32),
            pltpu.VMEM((1, 2 * T, S), F32),
            pltpu.VMEM((NX, NB, T + 16, T), F32),
            pltpu.VMEM((NU, 2, T, T), F32),
            pltpu.VMEM((NX, 8, T), F32),
            pltpu.VMEM((NU, 2, T, M), BF),
            pltpu.VMEM((KS, M), BF),
            pltpu.VMEM((NX, T), BF),
            pltpu.VMEM((NX, T), BF),
            pltpu.SemaphoreType.DMA((NU,)),
            pltpu.SemaphoreType.DMA,
            pltpu.SemaphoreType.DMA((2,)),
            pltpu.SemaphoreType.DMA((2,)),
            pltpu.SemaphoreType.DMA,
        ],
        compiler_params=pltpu.CompilerParams(vmem_limit_bytes=124 * 2**20),
        name="gated_mix_cla_h3",
    )(
        A_x.reshape(NU, 2, T, M), A_c_kv.reshape(NU, 2, T, Dc), A_w_q, A_w_uk, A_w_uv,
        A_w_o, B_k.reshape(S, M), B_v.reshape(S, M), B_ssm_k.reshape(NX, T, S),
        _dft_matrices(), B_shift_k.T, B_ssm_D.reshape(NX, T), gate_w.reshape(NX, T),
    )
    return out.reshape(B, S, M)
```
